```python
import jax
import jax.numpy as jnp

def _softmax(x, axis=-1):
    return jax.nn.softmax(x, axis=axis)
def _gelu(x):
    return jax.nn.gelu(x, approximate=True)
def _silu(x):
    return jax.nn.silu(x)
def _sigmoid(x):
    return jax.nn.sigmoid(x)
def _layernorm(x, axis=-1, eps=1e-5):
    m = jnp.mean(x, axis=axis, keepdims=True)
    v = jnp.var(x, axis=axis, keepdims=True)
    return (x - m) / jnp.sqrt(v + eps)
def _scatter_add(tgt, idx, src, axis=0):
    return tgt.at[idx].add(src)
def _segment_sum(src, seg, n):
    return jax.ops.segment_sum(src, seg, n)
class _Rng:
    def __init__(self, key):
        self._k = key
    def _next(self):
        self._k, sub = jax.random.split(self._k)
        return sub
    def normal(self, shape):
        return jax.random.normal(self._next(), shape, dtype=jnp.bfloat16)
    def randint(self, lo, hi, shape):
        return jax.random.randint(self._next(), shape, lo, hi, dtype=jnp.int32)
    def uniform(self, shape, lo=0.0, hi=1.0):
        return jax.random.uniform(self._next(), shape, jnp.bfloat16, lo, hi)
    def permutation(self, n):
        return jax.random.permutation(self._next(), n)


kernel_name = 'gated_mix__compressed_kv_cla__moe_arch_mod__prompt'

def setup_inputs():
    _rng = _Rng(jax.random.key(int.from_bytes(__import__("os").urandom(4), "little")))
    _w = (lambda a: (lambda t: t.astype(jnp.bfloat16) if jnp.issubdtype(t.dtype, jnp.floating) else t)(jnp.asarray(a)))
    def _A_setup():
        B, H, Sq, Sk, D, M = 1, 16, 2048, 2048, 256, 448
        Dc = 4 * D
        return {
            "x": _w((lambda *s: _rng.normal(s) * 0.05)(B, Sq, M)),
            "c_kv": _w((lambda *s: _rng.normal(s) * 0.05)(B, Sk, Dc)),
            "w_q": _w((lambda *s: _rng.normal(s) * 0.05)(M, H, D) * (M ** -0.5)),
            "w_uk": _w((lambda *s: _rng.normal(s) * 0.05)(Dc, H, D) * (Dc ** -0.5)),
            "w_uv": _w((lambda *s: _rng.normal(s) * 0.05)(Dc, H, D) * (Dc ** -0.5)),
            "w_o": _w((lambda *s: _rng.normal(s) * 0.05)(H, D, M) * ((H * D) ** -0.5)),
        }
    _A_in = _A_setup()

    def _B_setup():
        B, S, D, F, C = 1, 2048, 448, 1792, 2
        return {
            "x": _w((lambda *s: _rng.normal(s) * 0.05)(B, S, D)),
            "w_r": _w((lambda *s: _rng.normal(s) * 0.05)(D)),
            "w_gate": _w((lambda *s: _rng.normal(s) * 0.05)(D, F)),
            "w_up": _w((lambda *s: _rng.normal(s) * 0.05)(D, F)),
            "w_down": _w((lambda *s: _rng.normal(s) * 0.05)(F, D)),
        }
    _B_in = _B_setup()

    return {
        "A_x": _A_in["x"],
        "A_c_kv": _A_in["c_kv"],
        "A_w_q": _A_in["w_q"],
        "A_w_uk": _A_in["w_uk"],
        "A_w_uv": _A_in["w_uv"],
        "A_w_o": _A_in["w_o"],
        "B_x": _B_in["x"],
        "B_w_r": _B_in["w_r"],
        "B_w_gate": _B_in["w_gate"],
        "B_w_up": _B_in["w_up"],
        "B_w_down": _B_in["w_down"],
        "gate_w": _w((lambda *s: _rng.normal(s) * 0.05)(448)),
    }

def reference(A_x, A_c_kv, A_w_q, A_w_uk, A_w_uv, A_w_o, B_x, B_w_r, B_w_gate, B_w_up, B_w_down, gate_w):
    def _A_ref(x, c_kv, w_q, w_uk, w_uv, w_o):
        B, Sq, M = x.shape[0], x.shape[1], x.shape[2]
        Sk = c_kv.shape[1]
        H, D = w_q.shape[1], w_q.shape[2]
        q = jnp.einsum("bqm,mhd->bhqd", x, w_q)
        k = jnp.einsum("bkc,chd->bhkd", c_kv, w_uk)
        v = jnp.einsum("bkc,chd->bhkd", c_kv, w_uv)
        scores = jnp.einsum("bhqd,bhkd->bhqk", q, k) * (D ** -0.5)
        off = Sk - Sq
        qi = jnp.arange(Sq)[:, None]
        kj = jnp.arange(Sk)[None, :]
        cmask = kj <= (qi + off)
        scores = jnp.where(cmask[None, None], scores, -1e9)
        p = _softmax(scores, axis=-1)
        ctx = jnp.einsum("bhqk,bhkd->bhqd", p, v)
        return jnp.einsum("bhqd,hdm->bqm", ctx, w_o)

    def _B_ref(x, w_r, w_gate, w_up, w_down):
        B, S, D = x.shape
        C = 2
        r = x @ w_r
        idx = jnp.argsort(-r, axis=-1)[:, :C]
        idx_e = jnp.repeat(idx.reshape(B, C, 1), D, axis=2)
        x_sel = jnp.take_along_axis(x, idx_e, axis=1)
        g = _silu(x_sel @ w_gate)
        u = x_sel @ w_up
        y = (g * u) @ w_down
        r_sel = _sigmoid(jnp.take_along_axis(r, idx, axis=1))
        y = y * r_sel.reshape(B, C, 1)
        b_off = (jnp.arange(B) * S).reshape(B, 1)
        flat_idx = (idx + b_off).reshape(B * C)
        zero = (x * 0.0).reshape(B * S, D)
        upd = _scatter_add(zero, flat_idx, y.reshape(B * C, D), axis=0)
        return x + upd.reshape(B, S, D)

    x = A_x
    g = _sigmoid((x * gate_w).sum(-1, keepdims=True))
    a = _A_ref(x, A_c_kv, A_w_q, A_w_uk, A_w_uv, A_w_o)
    b = _B_ref(x, B_w_r, B_w_gate, B_w_up, B_w_down)
    return g * a + (1 - g) * b
```

```python
import functools
import math

import jax
import jax.numpy as jnp
from jax import lax
import jax.experimental.pallas as pl
import jax.experimental.pallas.tpu as pltpu

F32 = jnp.float32
BF16 = jnp.bfloat16
NT = (((1,), (1,)), ((), ()))

BQ = 128
OC = 512


def _dot(a, b):
    return jnp.dot(a, b, preferred_element_type=F32)


def _dot_nt(a, b):
    return lax.dot_general(a, b, NT, preferred_element_type=F32)


def _head_of_pair(w32, parity):
    sh = (16 * (1 - parity)).astype(jnp.uint32) if not isinstance(parity, int) else jnp.uint32(16 * (1 - parity))
    return pltpu.bitcast((w32 << sh) & jnp.uint32(0xFFFF0000), F32)


def _kernel(wr_ref, gw_ref, xT_hbm, c_hbm, wq_hbm, wk_hbm, wv_hbm, woT_hbm, wg_hbm, wu_hbm, wdT_hbm,
            outT_hbm,
            xT, c, wq32, wk32, wv32, woT, wg, wu, wdT,
            qT_all, wqT_buf, wk_buf, wvT_buf, k_buf, vT_buf, g_buf, y_buf, sel_buf, out_buf,
            sem_x, sem_c, sem_q, sem_k, sem_v, sem_o, sem_f, sem_out):
    M, S = xT.shape
    H = woT_hbm.shape[0]
    D = woT_hbm.shape[2]
    NP = H // 2
    NQ = S // BQ

    wq_h32 = wq_hbm.bitcast(jnp.uint32)
    wk_h32 = wk_hbm.bitcast(jnp.uint32)
    wv_h32 = wv_hbm.bitcast(jnp.uint32)

    cp_x = pltpu.make_async_copy(xT_hbm, xT, sem_x)
    cp_c = pltpu.make_async_copy(c_hbm, c, sem_c)
    cp_q = lambda j: pltpu.make_async_copy(wq_h32.at[:, j, :], wq32.at[j], sem_q.at[j])
    cp_k = lambda j: pltpu.make_async_copy(wk_h32.at[:, j, :], wk32.at[j], sem_k.at[j])
    cp_v = lambda j: pltpu.make_async_copy(wv_h32.at[:, j, :], wv32.at[j], sem_v.at[j])
    cp_o = lambda h: pltpu.make_async_copy(woT_hbm.at[h], woT.at[:, pl.ds(h * D, D)], sem_o.at[h])
    cp_f = [pltpu.make_async_copy(wg_hbm, wg, sem_f.at[0]),
            pltpu.make_async_copy(wu_hbm, wu, sem_f.at[1]),
            pltpu.make_async_copy(wdT_hbm, wdT, sem_f.at[2])]

    cp_q(0).start()
    cp_x.start()
    cp_q(1).start()

    qscale = (D ** -0.5) * math.log2(math.e)

    def prep_q(j, slot):
        w = wq32[j]
        for par in range(2):
            wqT_buf[slot, pl.ds(par * D, D), :] = _head_of_pair(w, par).T.astype(BF16)

    cp_q(0).wait()
    prep_q(0, 0)
    cp_x.wait()
    for j in range(2, NP):
        cp_q(j).start()
    cp_c.start()
    cp_k(0).start()
    cp_v(0).start()
    for cp in cp_f:
        cp.start()
    for j in range(1, NP):
        cp_k(j).start()
        cp_v(j).start()
    for h in range(H):
        cp_o(h).start()

    def q_body(j, _):
        @pl.when(j + 1 < NP)
        def _():
            cp_q(j + 1).wait()
        prep_q(jnp.minimum(j + 1, NP - 1), (j + 1) % 2)
        q = _dot(wqT_buf[j % 2], xT[...]) * qscale
        qT_all[pl.ds(pl.multiple_of(j * 2 * D, 2 * D), 2 * D), :] = q.astype(BF16)

    lax.fori_loop(0, NP, q_body, None)

    rows = lax.broadcasted_iota(jnp.int32, (16, M), 0)
    wr = wr_ref[...].astype(F32).reshape(1, M)
    gw = gw_ref[...].astype(F32).reshape(1, M)
    lhs = jnp.where(rows == 0, wr, jnp.where(rows == 1, gw, 0.0)).astype(BF16)
    rg = _dot(lhs, xT[...])
    r = rg[0:1, :].astype(BF16).astype(F32)
    g_buf[...] = jax.nn.sigmoid(rg[1:2, :])
    tok = lax.broadcasted_iota(jnp.int32, (1, S), 1)
    key = jnp.where(r != r, -jnp.inf, r)
    m1 = jnp.max(key, axis=1, keepdims=True)
    i1 = jnp.min(jnp.where(key == m1, tok, S), axis=1, keepdims=True)
    key2 = jnp.where(tok == i1, -jnp.inf, key)
    m2 = jnp.max(key2, axis=1, keepdims=True)
    i2 = jnp.min(jnp.where((key2 == m2) & (tok != i1), tok, S), axis=1, keepdims=True)
    sel_buf[0:1, :] = (tok == i1).astype(F32)
    sel_buf[1:2, :] = (tok == i2).astype(F32)
    rows_s = lax.broadcasted_iota(jnp.int32, (16, S), 0)
    onehot = jnp.where(rows_s == 0, (tok == i1).astype(F32), jnp.where(rows_s == 1, (tok == i2).astype(F32), 0.0))
    x_sel = _dot_nt(onehot.astype(BF16), xT[...]).astype(BF16)
    for cp in cp_f:
        cp.wait()
    gate = _dot(x_sel, wg[...])
    up = _dot(x_sel, wu[...])
    hid = (gate * jax.nn.sigmoid(gate) * up).astype(BF16)
    y = _dot_nt(hid, wdT[...])
    y1 = y[0:1, :] * jax.nn.sigmoid(m1)
    y2 = y[1:2, :] * jax.nn.sigmoid(m2)
    y_buf[0] = jnp.broadcast_to(y1, (128, M)).T
    y_buf[1] = jnp.broadcast_to(y2, (128, M)).T

    def prep_kv(h, slot):
        j = h // 2
        par = h % 2
        wk_buf[slot] = _head_of_pair(wk32[j], par).astype(BF16)
        wvT_buf[slot] = _head_of_pair(wv32[j], par).T.astype(BF16)

    cp_k(0).wait()
    cp_v(0).wait()
    prep_kv(0, 0)
    cp_c.wait()

    tri = (lax.broadcasted_iota(jnp.int32, (BQ, BQ), 0) <= lax.broadcasted_iota(jnp.int32, (BQ, BQ), 1))

    def head_body(h, _):
        @pl.when(jnp.logical_and(h % 2 == 1, h + 1 < H))
        def _():
            cp_k((h + 1) // 2).wait()
            cp_v((h + 1) // 2).wait()
        slot = h % 2
        hrows = pl.ds(pl.multiple_of(h * D, D), D)
        k_buf[...] = _dot(c[...], wk_buf[slot]).astype(BF16)
        vT_buf[...] = _dot_nt(wvT_buf[slot], c[...]).astype(BF16)
        prep_kv(jnp.minimum(h + 1, H - 1), 1 - slot)

        def scores(i):
            n = (i + 1) * BQ
            return _dot(k_buf[0:n, :], qT_all[hrows, i * BQ:(i + 1) * BQ])

        def softmax(i, s):
            n = i * BQ
            diag = jnp.where(tri, s[n:, :], -1e9 * math.log2(math.e))
            s = jnp.concatenate([s[:n, :], diag], axis=0) if i > 0 else diag
            m = jnp.max(s, axis=0, keepdims=True)
            p = jnp.exp2(s - m)
            l = jnp.sum(p, axis=0, keepdims=True)
            return p.astype(BF16), l

        def context(i, p, l):
            n = (i + 1) * BQ
            o = _dot(vT_buf[:, 0:n], p)
            qT_all[hrows, i * BQ:(i + 1) * BQ] = (o * (1.0 / l)).astype(BF16)

        order = list(range(NQ))[::-1]
        s_next = scores(order[0])
        for t, i in enumerate(order):
            s_cur = s_next
            if t + 1 < NQ:
                s_next = scores(order[t + 1])
            p, l = softmax(i, s_cur)
            context(i, p, l)

    lax.fori_loop(0, H, head_body, None)

    for h in range(H):
        cp_o(h).wait()
    NC = S // OC

    def cp_out(t):
        cols = pl.ds(pl.multiple_of(t * OC, OC), OC)
        return pltpu.make_async_copy(out_buf.at[t], outT_hbm.at[:, cols], sem_out.at[t])

    def out_body(t, _):
        cols = pl.ds(pl.multiple_of(t * OC, OC), OC)
        a = _dot(woT[...], qT_all[:, cols])
        g = g_buf[:, cols]
        s1 = sel_buf[0:1, cols] > 0.5
        s2 = sel_buf[1:2, cols] > 0.5
        y1 = jnp.concatenate([y_buf[0]] * (OC // 128), axis=1)
        y2 = jnp.concatenate([y_buf[1]] * (OC // 128), axis=1)
        b = xT[:, cols].astype(F32) + jnp.where(s1, y1, jnp.where(s2, y2, 0.0))
        out_buf[t] = (g * a + (1.0 - g) * b).astype(BF16)
        cp_out(t).start()

    lax.fori_loop(0, NC, out_body, None)
    for t in range(NC):
        cp_out(t).wait()


@jax.jit
def pallas_gated_mix__compressed_kv_cla__moe_arch_mod__prompt_kernel(
    A_x, A_c_kv, A_w_q, A_w_uk, A_w_uv, A_w_o, B_x, B_w_r, B_w_gate, B_w_up, B_w_down, gate_w,
):
    del B_x
    B, S, M = A_x.shape
    Dc = A_c_kv.shape[2]
    H, D = A_w_q.shape[1:]
    Fh = B_w_gate.shape[1]
    assert B == 1 and A_c_kv.shape[1] == S
    NP = H // 2
    hbm = pl.BlockSpec(memory_space=pl.ANY)
    vmem = pl.BlockSpec(memory_space=pltpu.VMEM)
    dma = pltpu.SemaphoreType.DMA
    outT = pl.pallas_call(
        _kernel,
        out_shape=jax.ShapeDtypeStruct((M, S), BF16),
        in_specs=[vmem, vmem] + [hbm] * 9,
        out_specs=hbm,
        scratch_shapes=[
            pltpu.VMEM((M, S), BF16),
            pltpu.VMEM((S, Dc), BF16),
            pltpu.VMEM((NP, M, D), jnp.uint32),
            pltpu.VMEM((NP, Dc, D), jnp.uint32),
            pltpu.VMEM((NP, Dc, D), jnp.uint32),
            pltpu.VMEM((M, H * D), BF16),
            pltpu.VMEM((M, Fh), BF16),
            pltpu.VMEM((M, Fh), BF16),
            pltpu.VMEM((M, Fh), BF16),
            pltpu.VMEM((H * D, S), BF16),
            pltpu.VMEM((2, 2 * D, M), BF16),
            pltpu.VMEM((2, Dc, D), BF16),
            pltpu.VMEM((2, D, Dc), BF16),
            pltpu.VMEM((S, D), BF16),
            pltpu.VMEM((D, S), BF16),
            pltpu.VMEM((1, S), F32),
            pltpu.VMEM((2, M, 128), F32),
            pltpu.VMEM((2, S), F32),
            pltpu.VMEM((S // OC, M, OC), BF16),
            dma, dma, dma((NP,)), dma((NP,)), dma((NP,)), dma((H,)), dma((3,)), dma((S // OC,)),
        ],
        compiler_params=pltpu.CompilerParams(vmem_limit_bytes=110 * 1024 * 1024),
        name="gated_mix_cla_mod",
    )(B_w_r, gate_w, A_x[0].T, A_c_kv[0], A_w_q, A_w_uk, A_w_uv,
      jnp.transpose(A_w_o, (0, 2, 1)), B_w_gate, B_w_up, B_w_down.T)
    return outT.T[None]
```

```python
import math
import os

import jax
import jax.numpy as jnp
from jax import lax
import jax.experimental.pallas as pl
import jax.experimental.pallas.tpu as pltpu

F32 = jnp.float32
BF16 = jnp.bfloat16
U32 = jnp.uint32

BQ = 128
KA = int(os.environ.get("KA", "6"))
VL = int(os.environ.get("VL", "1"))
CL = int(os.environ.get("CL", "2"))
XCH = tuple(int(v) for v in os.environ.get("XCH", "384,1152,2048").split(","))
OC = int(os.environ.get("OC", "512"))
OS = int(os.environ.get("OS", "128"))
XH = int(os.environ.get("XH", "0"))
ORD = os.environ.get("ORD", "skvc")
SCOPE = int(os.environ.get("SCOPE", "0"))


def _dot(a, b):
    return jnp.dot(a, b, preferred_element_type=F32)


def _dot_nt(a, b):
    return lax.dot_general(a, b, (((1,), (1,)), ((), ())), preferred_element_type=F32)


def _b(words):
    return pltpu.bitcast(words, BF16)


def _w(x):
    return pltpu.bitcast(x.astype(BF16), U32)


def _head_of_pair(w32, parity):
    if isinstance(parity, int):
        return pltpu.bitcast(w32 & jnp.uint32(0xFFFF0000) if parity else w32 << 16, F32)
    shift = (16 - 16 * parity).astype(U32)
    return pltpu.bitcast((w32 << shift) & jnp.uint32(0xFFFF0000), F32)


def _wait(name, copies):
    if SCOPE:
        with jax.named_scope("sc_" + name):
            for cp in copies:
                cp.wait()
    else:
        for cp in copies:
            cp.wait()


def _kernel(wr_hbm, gw_hbm, xT_hbm, c_hbm, wq_hbm, wk_hbm, wv_hbm, woT_hbm, wg_hbm, wu_hbm, wdT_hbm,
            outT_hbm,
            wr_ref, gw_ref, xT, c, wq32, wk32, wv32, woT, wg, wu, wdT,
            qT_all, wqT_buf, wk_buf, wvT_buf, k_buf, vT_buf, g_buf, sel_buf, out_buf, s_buf, zero_ref,
            sem_x, sem_q, sem_kv, sem):
    M, S = xT_hbm.shape
    H, _, D = woT_hbm.shape
    NP = H // 2
    NQ = S // BQ
    FC = wg.shape[2]

    copy = pltpu.make_async_copy
    xT_h32 = xT_hbm.bitcast(U32)
    wq_h32 = wq_hbm.bitcast(U32)
    wk_h32 = wk_hbm.bitcast(U32)
    wv_h32 = wv_hbm.bitcast(U32)
    ffn = [(wg_hbm.bitcast(U32), wg), (wu_hbm.bitcast(U32), wu), (wdT_hbm.bitcast(U32), wdT)]

    x_chunks = list(zip((0,) + XCH[:-1], XCH))
    cp_x = [[copy(xT_h32.at[:, a:b], xT.at[:, a:b], sem_x.at[t])] for t, (a, b) in enumerate(x_chunks)]
    cp_x[-1] += [copy(wq_h32.at[:, 1, :], wq32.at[1], sem_x.at[len(XCH) - 1]),
                 copy(wr_hbm, wr_ref, sem_x.at[len(XCH) - 1]), copy(gw_hbm, gw_ref, sem_x.at[len(XCH) - 1])]
    cp_q0 = copy(wq_h32.at[:, 0, :], wq32.at[0], sem.at[0])

    def cp_ffn(t):
        cols = pl.ds(t * FC if isinstance(t, int) else pl.multiple_of(t * FC, FC), FC)
        return [copy(src.at[:, cols], dst.at[t], sem_q.at[t]) for src, dst in ffn]

    def cp_q(t):
        return [copy(wq_h32.at[:, t + 2, :], wq32.at[t + 2], sem_q.at[t])]

    def cp_kv(j):
        return [copy(wk_h32.at[:, j, :], wk32.at[j], sem_kv.at[j]), copy(wv_h32.at[:, j, :], wv32.at[j], sem_kv.at[j])]

    cp_c = copy(c_hbm.bitcast(U32), c, sem_kv.at[0])
    cp_o = copy(woT_hbm.bitcast(U32), woT, sem.at[1])

    cp_q0.start()
    for cps in cp_x:
        for cp in cps:
            cp.start()

    qscale = (D ** -0.5) * math.log2(math.e)

    def wq_pair(j):
        w = wq32[j]
        return jnp.concatenate([_head_of_pair(w, par).T for par in range(2)], axis=0)

    zero_ref[0] = 0
    _wait("q0", [cp_q0])
    w0 = wq_pair(0).astype(BF16)
    for t, (a, b) in enumerate(x_chunks):
        _wait("x", cp_x[t])
        if t == len(x_chunks) - 1:
            for i in range(NP - 1):
                for cp in cp_ffn(i) + (cp_q(i) if i + 2 < NP else []):
                    cp.start()
            cp_c.start()
            for j in range(NP):
                for cp in cp_kv(j):
                    cp.start()
            cp_o.start()
            rows = lax.broadcasted_iota(jnp.int32, (16, M), 0)
            wr = wr_ref[...].astype(F32).reshape(1, M)
            gw = gw_ref[...].astype(F32).reshape(1, M)
            lhs = jnp.where(rows == 0, wr, jnp.where(rows == 1, gw, 0.0)).astype(BF16)
            rg = _dot(lhs, _b(xT[...]))
        qT_all[0:D, a:b] = _w(_dot(w0, _b(xT[:, a:b])) * qscale)
    wqT_buf[...] = _w(wq_pair(1))

    r = rg[0:1, :].astype(BF16).astype(F32)
    g_buf[...] = jax.nn.sigmoid(rg[1:2, :])
    tok = lax.broadcasted_iota(jnp.int32, (1, S), 1)
    key = jnp.where(r != r, -jnp.inf, r)
    m1 = jnp.max(key, axis=1, keepdims=True)
    i1 = jnp.min(jnp.where(key == m1, tok, S), axis=1, keepdims=True)
    key2 = jnp.where(tok == i1, -jnp.inf, key)
    m2 = jnp.max(key2, axis=1, keepdims=True)
    i2 = jnp.min(jnp.where((key2 == m2) & (tok != i1), tok, S), axis=1, keepdims=True)
    sel_buf[0:1, :] = (tok == i1).astype(F32)
    sel_buf[1:2, :] = (tok == i2).astype(F32)
    lane = lax.broadcasted_iota(jnp.int32, (M // 2, 128), 1)
    picked = []
    for idx in (i1, i2):
        acc = jnp.zeros((M // 2, 128), U32)
        for t in range(S // 128):
            acc = jnp.where(lane == idx - t * 128, xT[:, t * 128:(t + 1) * 128], acc)
        picked.append(acc)
    half = lax.broadcasted_iota(jnp.int32, (16, 256), 1) // 128
    pick = (half == lax.broadcasted_iota(jnp.int32, (16, 256), 0)).astype(F32).astype(BF16)
    x_sel = _dot_nt(pick, _b(jnp.concatenate(picked, axis=1)))

    def q_body(t, y):
        _wait("f", cp_ffn(t))

        @pl.when(t + 2 < NP)
        def _():
            _wait("q", cp_q(t))

        hrows = pl.ds(pl.multiple_of((t + 1) * D, D), D)
        xs = x_sel.astype(BF16)
        nf = FC // 128
        parts, hid = [], []
        for i in range(S // 128):
            cols = slice(i * 128, (i + 1) * 128)
            qT_all[hrows, cols] = _w(_dot(_b(wqT_buf[...]), _b(xT[:, cols])) * qscale)
            if i < 2 * nf:
                f = i // 2
                parts.append(_dot(xs, _b((wu if i % 2 else wg)[t, :, f * 128:(f + 1) * 128])))
                if i % 2:
                    hid.append((parts[-2] * jax.nn.sigmoid(parts[-2]) * parts[-1]).astype(BF16))
            elif i < 3 * nf:
                f = i - 2 * nf
                y = y + _dot_nt(hid[f], _b(wdT[t, :, f * 128:(f + 1) * 128]))
        wqT_buf[...] = _w(wq_pair(jnp.minimum(t + 2, NP - 1)))
        return y

    y = lax.fori_loop(0, NP - 1, q_body, jnp.zeros((16, M), F32))
    y1 = y[0:1, :] * jax.nn.sigmoid(m1)
    y2 = y[1:2, :] * jax.nn.sigmoid(m2)

    _wait("c", [cp_c] + cp_kv(0))
    wk_buf[...] = _w(_head_of_pair(wk32[0], 0))
    zr = pl.ds(pl.multiple_of(zero_ref[0] * 8, 8), 8)
    for ref in (k_buf, vT_buf, wvT_buf):
        ref[zr, 0:128] = jnp.zeros((8, 128), U32)

    def head_body(it, _):
        @pl.when(jnp.logical_and(it % 2 == 1, it + 1 < H))
        def _():
            _wait("kv", cp_kv((it + 1) // 2))

        h = jnp.minimum(it, H - 1) if XH else it
        nxt = jnp.minimum(h + 1, H - 1)
        zero = zero_ref[0]
        tri = (lax.broadcasted_iota(jnp.int32, (BQ, BQ), 0) <= lax.broadcasted_iota(jnp.int32, (BQ, BQ), 1))
        hrows = pl.ds(pl.multiple_of(h * (D // 2), D // 2), D // 2)

        def proj_k(a, b):
            k_buf[a // 2:b // 2, :] = _w(_dot(_b(c[a // 2:b // 2, :]), _b(wk_buf[...])))

        def proj_v(a, b):
            vT_buf[:, a:b] = _w(_dot_nt(_b(wvT_buf[...]), _b(c[a // 2:b // 2, :])))

        def scores(i):
            n = (i + 1) * BQ
            s = _dot(_b(k_buf[0:n // 2, :]), _b(qT_all[hrows, i * BQ:n]))
            diag = jnp.where(tri, s[n - BQ:, :], -1e9 * math.log2(math.e))
            s = jnp.concatenate([s[:n - BQ, :], diag], axis=0) if i > 0 else diag
            s_buf[i][zero] = s
            return jnp.max(s, axis=0, keepdims=True)

        def context(i, m):
            n = (i + 1) * BQ
            p = jnp.exp2(s_buf[i][0] - m)
            l = jnp.sum(p, axis=0, keepdims=True)
            o = _dot(_b(vT_buf[:, 0:n]), p.astype(BF16))
            qT_all[hrows, i * BQ:n] = _w(o * (1.0 / l))

        row_max = {}
        wvT_buf[...] = _w(_head_of_pair(wv32[h // 2], h % 2).T)
        proj_k(0, KA * BQ)
        for step in range(NQ + CL):
            for op in ORD:
                i = step + {"s": 0, "k": KA, "v": -VL, "c": -CL}[op]
                if not 0 <= i < NQ:
                    continue
                if op == "s":
                    row_max[i] = scores(i)
                elif op == "k":
                    proj_k(i * BQ, (i + 1) * BQ)
                    if i == NQ - 1:
                        wk_buf[...] = _w(_head_of_pair(wk32[nxt // 2], nxt % 2))
                elif op == "v":
                    proj_v(i * BQ, (i + 1) * BQ)
                else:
                    context(i, row_max.pop(i))

    lax.fori_loop(0, H + XH, head_body, None)

    _wait("o", [cp_o])

    def cp_out(t, a, b):
        cols = pl.ds(t * OC + a if isinstance(t, int) else pl.multiple_of(t * OC + a, 128), b - a)
        return copy(out_buf.at[t, :, pl.ds(a, b - a)], outT_hbm.at[:, cols], sem.at[2])

    pieces = [(0, OC - OS), (OC - OS, OC)] if OS else [(0, OC)]

    def out_body(t, _):
        y1c = jnp.broadcast_to(y1, (128, M)).T
        y2c = jnp.broadcast_to(y2, (128, M)).T
        for a, b in pieces:
            cols = pl.ds(pl.multiple_of(t * OC + a, 128), b - a)
            wo = jnp.concatenate([_b(woT[h]) for h in range(H)], axis=1)
            att = _dot(wo, _b(qT_all[:, cols]))
            g = g_buf[:, cols]
            s1 = sel_buf[0:1, cols] > 0.5
            s2 = sel_buf[1:2, cols] > 0.5
            rep = (b - a) // 128
            upd = jnp.where(s1, jnp.concatenate([y1c] * rep, axis=1),
                            jnp.where(s2, jnp.concatenate([y2c] * rep, axis=1), 0.0))
            res = _b(xT[:, cols]).astype(F32) + upd
            out_buf[t, :, a:b] = (g * att + (1.0 - g) * res).astype(BF16)
            cp_out(t, a, b).start()

    lax.fori_loop(0, S // OC, out_body, None)
    _wait("out", [cp_out(t, a, b) for t in range(S // OC) for a, b in pieces])


@jax.jit
def pallas_gated_mix__compressed_kv_cla__moe_arch_mod__prompt_kernel(
    A_x, A_c_kv, A_w_q, A_w_uk, A_w_uv, A_w_o, B_x, B_w_r, B_w_gate, B_w_up, B_w_down, gate_w,
):
    del B_x
    B, S, M = A_x.shape
    Dc = A_c_kv.shape[2]
    H, D = A_w_q.shape[1:]
    Fh = B_w_gate.shape[1]
    assert B == 1 and A_c_kv.shape[1] == S
    NP = H // 2
    FC = Fh // (NP - 1)
    hbm = pl.BlockSpec(memory_space=pl.ANY)
    dma = pltpu.SemaphoreType.DMA
    outT = pl.pallas_call(
        _kernel,
        out_shape=jax.ShapeDtypeStruct((M, S), BF16),
        in_specs=[hbm] * 11,
        out_specs=hbm,
        scratch_shapes=[
            pltpu.VMEM((M,), BF16),
            pltpu.VMEM((M,), BF16),
            pltpu.VMEM((M // 2, S), U32),
            pltpu.VMEM((S // 2, Dc), U32),
            pltpu.VMEM((NP, M, D), U32),
            pltpu.VMEM((NP, Dc, D), U32),
            pltpu.VMEM((NP, Dc, D), U32),
            pltpu.VMEM((H, M // 2, D), U32),
            pltpu.VMEM((NP - 1, M // 2, FC), U32),
            pltpu.VMEM((NP - 1, M // 2, FC), U32),
            pltpu.VMEM((NP - 1, M // 2, FC), U32),
            pltpu.VMEM((H * D // 2, S), U32),
            pltpu.VMEM((D, M), U32),
            pltpu.VMEM((Dc // 2, D), U32),
            pltpu.VMEM((D // 2, Dc), U32),
            pltpu.VMEM((S // 2, D), U32),
            pltpu.VMEM((D // 2, S), U32),
            pltpu.VMEM((1, S), F32),
            pltpu.VMEM((2, S), F32),
            pltpu.VMEM((S // OC, M, OC), BF16),
            [pltpu.VMEM((1, (i + 1) * BQ, BQ), F32) for i in range(S // BQ)],
            pltpu.SMEM((1,), jnp.int32),
            dma((len(XCH),)), dma((NP - 1,)), dma((NP,)), dma((3,)),
        ],
        compiler_params=pltpu.CompilerParams(vmem_limit_bytes=110 * 1024 * 1024),
        name="gated_mix_cla_mod",
    )(B_w_r, gate_w, A_x[0].T, A_c_kv[0], A_w_q, A_w_uk, A_w_uv,
      jnp.transpose(A_w_o, (0, 2, 1)), B_w_gate, B_w_up, B_w_down.T)
    return outT.T[None]
```

```python
import math

import jax
import jax.numpy as jnp
from jax import lax
import jax.experimental.pallas as pl
import jax.experimental.pallas.tpu as pltpu

F32 = jnp.float32
BF16 = jnp.bfloat16
U32 = jnp.uint32
LOG2E = math.log2(math.e)

BQ = 128
K_AHEAD, V_LAG, CTX_LAG = 4, 1, 3
X_CHUNKS = (384, 1152)
OUT_CHUNK, OUT_TAIL = 512, 128


def _dot(a, b):
    return jnp.dot(a, b, preferred_element_type=F32)


def _dot_nt(a, b):
    return lax.dot_general(a, b, (((1,), (1,)), ((), ())), preferred_element_type=F32)


def _bf16(words):
    return pltpu.bitcast(words, BF16)


def _words(x):
    return pltpu.bitcast(x.astype(BF16), U32)


def _head_of_pair(words, parity):
    if isinstance(parity, int):
        return pltpu.bitcast(words & jnp.uint32(0xFFFF0000) if parity else words << 16, F32)
    shift = (16 - 16 * parity).astype(U32)
    return pltpu.bitcast((words << shift) & jnp.uint32(0xFFFF0000), F32)


def _start(copies):
    for cp in copies:
        cp.start()


def _wait(copies):
    for cp in copies:
        cp.wait()


def _kernel(wr_hbm, gw_hbm, xT_hbm, c_hbm, wq_hbm, wk_hbm, wv_hbm, woT_hbm, wg_hbm, wu_hbm, wdT_hbm,
            outT_hbm,
            wr, gw, xT, c, wq, wk, wv, woT, wg, wu, wdT,
            qT, wqT_cur, wk_cur, wvT_cur, k_buf, vT_buf, s_buf, gate_buf, sel_buf, out_buf, zero_ref,
            sem_x, sem_q, sem):
    M, S = xT_hbm.shape
    H, _, D = woT_hbm.shape
    NP = H // 2
    NQ = S // BQ
    FC = wg.shape[2]

    copy = pltpu.make_async_copy
    xT_src, wq_src, wk_src, wv_src = (r.bitcast(U32) for r in (xT_hbm, wq_hbm, wk_hbm, wv_hbm))
    ffn = [(wg_hbm.bitcast(U32), wg), (wu_hbm.bitcast(U32), wu), (wdT_hbm.bitcast(U32), wdT)]

    x_chunks = list(zip((0,) + X_CHUNKS, X_CHUNKS + (S,)))
    cp_first = [copy(wq_src.at[:, 0, :], wq.at[0], sem.at[0]),
                copy(wr_hbm, wr, sem.at[0]), copy(gw_hbm, gw, sem.at[0])]
    cp_x = [[copy(xT_src.at[:, a:b], xT.at[:, a:b], sem_x.at[t])] for t, (a, b) in enumerate(x_chunks)]
    cp_x[-1].append(copy(wq_src.at[:, 1, :], wq.at[1], sem_x.at[len(X_CHUNKS)]))

    def cp_ffn(t):
        cols = pl.ds(t * FC if isinstance(t, int) else pl.multiple_of(t * FC, FC), FC)
        return [copy(src.at[:, cols], dst.at[t], sem_q.at[t]) for src, dst in ffn]

    def cp_wq(t):
        return [copy(wq_src.at[:, t + 2, :], wq.at[t + 2], sem_q.at[t])]

    cp_kv = [copy(c_hbm.bitcast(U32), c, sem.at[1])]
    for j in range(NP):
        cp_kv += [copy(wk_src.at[:, j, :], wk.at[j], sem.at[1]), copy(wv_src.at[:, j, :], wv.at[j], sem.at[1])]
    cp_wo = [copy(woT_hbm.bitcast(U32), woT, sem.at[2])]

    _start(cp_first)
    for cps in cp_x:
        _start(cps)
    for t in range(NP - 1):
        _start(cp_ffn(t) + (cp_wq(t) if t + 2 < NP else []))
    _start(cp_kv + cp_wo)
    zero_ref[0] = 0

    q_scale = (D ** -0.5) * LOG2E

    def wqT_pair(j):
        return jnp.concatenate([_head_of_pair(wq[j], par).T for par in range(2)], axis=0)

    _wait(cp_first)
    row = lax.broadcasted_iota(jnp.int32, (16, M), 0)
    w_rg = jnp.where(row == 0, wr[...].astype(F32).reshape(1, M),
                     jnp.where(row == 1, gw[...].astype(F32).reshape(1, M), 0.0)).astype(BF16)
    w_first = wqT_pair(0).astype(BF16)
    rg = []
    for t, (a, b) in enumerate(x_chunks):
        _wait(cp_x[t])
        if b < S:
            q = _dot(jnp.concatenate([w_first, w_rg], axis=0), _bf16(xT[:, a:b]))
            rg.append(q[2 * D:])
        else:
            rg.append(_dot(w_rg, _bf16(xT[:, a:b])))
            q = _dot(w_first, _bf16(xT[:, a:b]))
        qT[0:D, a:b] = _words(q[:2 * D] * q_scale)
    rg = jnp.concatenate(rg, axis=1)
    wqT_cur[...] = _words(wqT_pair(1))

    gate_buf[...] = jax.nn.sigmoid(rg[1:2, :])
    r = rg[0:1, :].astype(BF16).astype(F32)
    tok = lax.broadcasted_iota(jnp.int32, (1, S), 1)
    key1 = jnp.where(r != r, -jnp.inf, r)
    r1 = jnp.max(key1, axis=1, keepdims=True)
    i1 = jnp.min(jnp.where(key1 == r1, tok, S), axis=1, keepdims=True)
    key2 = jnp.where(tok == i1, -jnp.inf, key1)
    r2 = jnp.max(key2, axis=1, keepdims=True)
    i2 = jnp.min(jnp.where((key2 == r2) & (tok != i1), tok, S), axis=1, keepdims=True)
    sel_buf[0:1, :] = (tok == i1).astype(F32)
    sel_buf[1:2, :] = (tok == i2).astype(F32)
    lane = lax.broadcasted_iota(jnp.int32, (M // 2, 128), 1)
    picked = []
    for idx in (i1, i2):
        col = jnp.zeros((M // 2, 128), U32)
        for t in range(S // 128):
            col = jnp.where(lane == idx - t * 128, xT[:, t * 128:(t + 1) * 128], col)
        picked.append(col)
    half = lax.broadcasted_iota(jnp.int32, (16, 256), 1) // 128
    to_row = (half == lax.broadcasted_iota(jnp.int32, (16, 256), 0)).astype(F32).astype(BF16)
    x_sel = _dot_nt(to_row, _bf16(jnp.concatenate(picked, axis=1)))

    def q_body(t, y):
        _wait(cp_ffn(t))

        @pl.when(t + 2 < NP)
        def _():
            _wait(cp_wq(t))

        rows = pl.ds(pl.multiple_of((t + 1) * D, D), D)
        xs = x_sel.astype(BF16)
        nf = FC // 128
        gate_up, hidden = [], []
        for i in range(S // 128):
            cols = slice(i * 128, (i + 1) * 128)
            qT[rows, cols] = _words(_dot(_bf16(wqT_cur[...]), _bf16(xT[:, cols])) * q_scale)
            if i < 2 * nf:
                f = i // 2
                gate_up.append(_dot(xs, _bf16((wu if i % 2 else wg)[t, :, f * 128:(f + 1) * 128])))
                if i % 2:
                    g, u = gate_up[-2:]
                    hidden.append((g * jax.nn.sigmoid(g) * u).astype(BF16))
            elif i < 3 * nf:
                f = i - 2 * nf
                y = y + _dot_nt(hidden[f], _bf16(wdT[t, :, f * 128:(f + 1) * 128]))
        wqT_cur[...] = _words(wqT_pair(jnp.minimum(t + 2, NP - 1)))
        return y

    y = lax.fori_loop(0, NP - 1, q_body, jnp.zeros((16, M), F32))
    y1 = y[0:1, :] * jax.nn.sigmoid(r1)
    y2 = y[1:2, :] * jax.nn.sigmoid(r2)

    _wait(cp_kv)
    wk_cur[...] = _words(_head_of_pair(wk[0], 0))
    for ref in (k_buf, vT_buf, wvT_cur):
        ref[pl.ds(pl.multiple_of(zero_ref[0] * 8, 8), 8), 0:128] = jnp.zeros((8, 128), U32)

    def head_body(h, _):
        nxt = jnp.minimum(h + 1, H - 1)
        zero = zero_ref[0]
        rows = pl.ds(pl.multiple_of(h * (D // 2), D // 2), D // 2)
        visible = (lax.broadcasted_iota(jnp.int32, (BQ, BQ), 0)
                   <= lax.broadcasted_iota(jnp.int32, (BQ, BQ), 1))

        def project_k(a, b):
            k_buf[a // 2:b // 2, :] = _words(_dot(_bf16(c[a // 2:b // 2, :]), _bf16(wk_cur[...])))

        def project_v(a, b):
            vT_buf[:, a:b] = _words(_dot_nt(_bf16(wvT_cur[...]), _bf16(c[a // 2:b // 2, :])))

        def scores(i):
            n = (i + 1) * BQ
            s = _dot(_bf16(k_buf[0:n // 2, :]), _bf16(qT[rows, n - BQ:n]))
            diag = jnp.where(visible, s[n - BQ:, :], -1e9 * LOG2E)
            s = jnp.concatenate([s[:n - BQ, :], diag], axis=0) if i > 0 else diag
            s_buf[i][zero] = s
            return jnp.max(s, axis=0, keepdims=True)

        def context(i, m):
            n = (i + 1) * BQ
            p = jnp.exp2(s_buf[i][0] - m)
            l = jnp.sum(p, axis=0, keepdims=True)
            o = _dot(_bf16(vT_buf[:, 0:n]), p.astype(BF16))
            qT[rows, n - BQ:n] = _words(o * (1.0 / l))

        wvT_cur[...] = _words(_head_of_pair(wv[h >> 1], h & 1).T)
        project_k(0, K_AHEAD * BQ)
        row_max = {}
        for step in range(NQ + CTX_LAG):
            if step < NQ:
                row_max[step] = scores(step)
            i = step - V_LAG
            if 0 <= i < NQ:
                project_v(i * BQ, (i + 1) * BQ)
            i = step + K_AHEAD
            if i < NQ:
                project_k(i * BQ, (i + 1) * BQ)
            if i == NQ - 1:
                wk_cur[...] = _words(_head_of_pair(wk[nxt >> 1], nxt & 1))
            i = step - CTX_LAG
            if i >= 0:
                context(i, row_max.pop(i))

    lax.fori_loop(0, H, head_body, None)

    _wait(cp_wo)
    pieces = [(0, OUT_CHUNK - OUT_TAIL), (OUT_CHUNK - OUT_TAIL, OUT_CHUNK)]

    def out_cols(t, a, b):
        start = t * OUT_CHUNK + a
        return pl.ds(start if isinstance(t, int) else pl.multiple_of(start, 128), b - a)

    def cp_out(t, a, b):
        return copy(out_buf.at[t, :, pl.ds(a, b - a)], outT_hbm.at[:, out_cols(t, a, b)], sem.at[3])

    def out_body(t, _):
        y1_col = jnp.broadcast_to(y1, (128, M)).T
        y2_col = jnp.broadcast_to(y2, (128, M)).T
        for a, b in pieces:
            cols = out_cols(t, a, b)
            wo = jnp.concatenate([_bf16(woT[h]) for h in range(H)], axis=1)
            att = _dot(wo, _bf16(qT[:, cols]))
            rep = (b - a) // 128
            upd = jnp.where(sel_buf[0:1, cols] > 0.5, jnp.concatenate([y1_col] * rep, axis=1),
                            jnp.where(sel_buf[1:2, cols] > 0.5, jnp.concatenate([y2_col] * rep, axis=1), 0.0))
            res = _bf16(xT[:, cols]).astype(F32) + upd
            g = gate_buf[:, cols]
            out_buf[t, :, a:b] = (g * att + (1.0 - g) * res).astype(BF16)
            cp_out(t, a, b).start()

    lax.fori_loop(0, S // OUT_CHUNK, out_body, None)
    _wait([cp_out(t, a, b) for t in range(S // OUT_CHUNK) for a, b in pieces])


@jax.jit
def pallas_gated_mix__compressed_kv_cla__moe_arch_mod__prompt_kernel(
    A_x: jax.Array,
    A_c_kv: jax.Array,
    A_w_q: jax.Array,
    A_w_uk: jax.Array,
    A_w_uv: jax.Array,
    A_w_o: jax.Array,
    B_x: jax.Array,
    B_w_r: jax.Array,
    B_w_gate: jax.Array,
    B_w_up: jax.Array,
    B_w_down: jax.Array,
    gate_w: jax.Array,
):
    del B_x
    B, S, M = A_x.shape
    Dc = A_c_kv.shape[2]
    H, D = A_w_q.shape[1:]
    NP = H // 2
    FC = B_w_gate.shape[1] // (NP - 1)
    assert B == 1 and A_c_kv.shape[1] == S and S % OUT_CHUNK == 0 and S > X_CHUNKS[-1]
    assert FC * (NP - 1) == B_w_gate.shape[1] and FC % 128 == 0 and 3 * FC <= S
    hbm = pl.BlockSpec(memory_space=pl.ANY)
    vmem = pltpu.VMEM
    dma = pltpu.SemaphoreType.DMA
    outT = pl.pallas_call(
        _kernel,
        out_shape=jax.ShapeDtypeStruct((M, S), BF16),
        in_specs=[hbm] * 11,
        out_specs=hbm,
        scratch_shapes=[
            vmem((M,), BF16),
            vmem((M,), BF16),
            vmem((M // 2, S), U32),
            vmem((S // 2, Dc), U32),
            vmem((NP, M, D), U32),
            vmem((NP, Dc, D), U32),
            vmem((NP, Dc, D), U32),
            vmem((H, M // 2, D), U32),
            vmem((NP - 1, M // 2, FC), U32),
            vmem((NP - 1, M // 2, FC), U32),
            vmem((NP - 1, M // 2, FC), U32),
            vmem((H * D // 2, S), U32),
            vmem((D, M), U32),
            vmem((Dc // 2, D), U32),
            vmem((D // 2, Dc), U32),
            vmem((S // 2, D), U32),
            vmem((D // 2, S), U32),
            [vmem((1, (i + 1) * BQ, BQ), F32) for i in range(S // BQ)],
            vmem((1, S), F32),
            vmem((2, S), F32),
            vmem((S // OUT_CHUNK, M, OUT_CHUNK), BF16),
            pltpu.SMEM((1,), jnp.int32),
            dma((len(X_CHUNKS) + 1,)), dma((NP - 1,)), dma((4,)),
        ],
        compiler_params=pltpu.CompilerParams(vmem_limit_bytes=110 * 1024 * 1024),
        name="gated_mix_cla_mod",
    )(B_w_r, gate_w, A_x.reshape(S, M).T, A_c_kv.reshape(S, Dc), A_w_q, A_w_uk, A_w_uv,
      jnp.transpose(A_w_o, (0, 2, 1)), B_w_gate, B_w_up, B_w_down.T)
    return outT.T.reshape(B, S, M)
```
